```python
import os as _os
_os.environ.setdefault("JAX_PLATFORMS", "cpu")
import jax
import jax.numpy as jnp

def _softmax(x, axis=-1):
    return jax.nn.softmax(x, axis=axis)
def _gelu(x):
    return jax.nn.gelu(x, approximate=True)
def _silu(x):
    return jax.nn.silu(x)
def _sigmoid(x):
    return jax.nn.sigmoid(x)
def _layernorm(x, axis=-1, eps=1e-5):
    m = jnp.mean(x, axis=axis, keepdims=True)
    v = jnp.var(x, axis=axis, keepdims=True)
    return (x - m) / jnp.sqrt(v + eps)
def _scatter_add(tgt, idx, src, axis=0):
    return tgt.at[idx].add(src)
def _segment_sum(src, seg, n):
    return jax.ops.segment_sum(src, seg, n)
class _Rng:
    def __init__(self, key):
        self._k = key
    def _next(self):
        self._k, sub = jax.random.split(self._k)
        return sub
    def normal(self, shape):
        return jax.random.normal(self._next(), shape, dtype=jnp.bfloat16)
    def randint(self, lo, hi, shape):
        return jax.random.randint(self._next(), shape, lo, hi, dtype=jnp.int32)
    def uniform(self, shape, lo=0.0, hi=1.0):
        return jax.random.uniform(self._next(), shape, jnp.bfloat16, lo, hi)
    def permutation(self, n):
        return jax.random.permutation(self._next(), n)


kernel_name = 'gated_mix__linear_attn_block__mixer_token_mlp__prompt'

def setup_inputs():
    _rng = _Rng(jax.random.key(int.from_bytes(__import__("os").urandom(4), "little")))
    _w = (lambda a: (lambda t: t.astype(jnp.bfloat16) if jnp.issubdtype(t.dtype, jnp.floating) else t)(jnp.asarray(a)))
    def _A_setup():
        B, S, D = 1, 2048, 512
        return {
            "x": _w((lambda *s: _rng.normal(s) * 0.05)(B, S, D)),
            "wqkv": _w((lambda *s: _rng.normal(s) * 0.8)(D, 3 * D)),
            "wo": _w((lambda *s: _rng.normal(s) * 0.05)(D, D)),
        }
    _A_in = _A_setup()

    def _B_setup():
        B, S, D, F = 1, 2048, 512, 1792
        return {
            "x": _w((lambda *s: _rng.normal(s) * 0.05)(B, S, D)),
            "w1": _w((lambda *s: _rng.normal(s) * 0.1)(S, F) * (S ** -0.5)),
            "b1": _w((lambda *s: _rng.normal(s) * 0.1)(F) * 0.02),
            "w2": _w((lambda *s: _rng.normal(s) * 0.1)(F, S) * (F ** -0.5)),
            "b2": _w((lambda *s: _rng.normal(s) * 0.1)(S) * 0.02),
        }
    _B_in = _B_setup()

    return {
        "A_x": _A_in["x"],
        "A_wqkv": _A_in["wqkv"],
        "A_wo": _A_in["wo"],
        "B_x": _B_in["x"],
        "B_w1": _B_in["w1"],
        "B_b1": _B_in["b1"],
        "B_w2": _B_in["w2"],
        "B_b2": _B_in["b2"],
        "gate_w": _w((lambda *s: _rng.normal(s) * 0.05)(512) * 16.0),
    }

def reference(A_x, A_wqkv, A_wo, B_x, B_w1, B_b1, B_w2, B_b2, gate_w):
    def _A_ref(x, wqkv, wo):
        B, S, D = x.shape
        H = 32; Dh = D // H
        qkv = (lambda x, *d: x.transpose(*d))((x @ wqkv).reshape(B, S, 3, H, Dh), 2, 0, 3, 1, 4)
        q, k, v = qkv[0], qkv[1], qkv[2]
        phi = lambda t: jnp.where(t > 0, t + 1, jnp.exp(t)) + 1e-6
        pq, pk = phi(q), phi(k)
        kv = jnp.einsum("bhsd,bhse->bhde", pk, v)
        z = jnp.einsum("bhsd->bhd", pk)
        num = jnp.einsum("bhqd,bhde->bhqe", pq, kv)
        den = jnp.einsum("bhqd,bhd->bhq", pq, z)[..., None] + 1e-6
        o = num / den
        return (lambda x, *d: x.transpose(*d))(o, 0, 2, 1, 3).reshape(B, S, D) @ wo

    def _B_ref(x, w1, b1, w2, b2):
        B, S, D = x.shape
        h = _layernorm(x, axis=-1)
        u = jnp.einsum("bsd,sf->bdf", h, w1) + b1
        u = _gelu(u)
        y = jnp.einsum("bdf,fs->bds", u, w2) + b2
        return (lambda x, *d: x.transpose(*d))(y, 0, 2, 1)

    x = A_x
    g = _sigmoid((x * gate_w).sum(-1, keepdims=True))
    a = _A_ref(x, A_wqkv, A_wo)
    b = _B_ref(x, B_w1, B_b1, B_w2, B_b2)
    return g * a + (1 - g) * b
```

```python
import functools
import jax
import jax.numpy as jnp
import numpy as np
import jax.experimental.pallas as pl
import jax.experimental.pallas.tpu as pltpu

S, D, F, H = 2048, 512, 1792, 32
DH = D // H
CS = 512
NCS = S // CS
CF = 256
NCF = F // CF
CO = 256
NCO = S // CO

f32 = jnp.float32
bf16 = jnp.bfloat16
u32 = jnp.uint32
NT = (((1,), (1,)), ((), ()))


def _phi(t):
    return jnp.where(t > 0, t + 1.0, jnp.exp(t)) + 1e-6


def _gelu(x):
    c = np.float32(np.sqrt(2.0 / np.pi))
    return 0.5 * x * (1.0 + jnp.tanh(c * (x + 0.044715 * (x * x * x))))


def _dot(a, b):
    return jnp.dot(a, b, preferred_element_type=f32)


def _dot_nt(a, b):
    return jax.lax.dot_general(a, b, NT, preferred_element_type=f32)


def _pk(x):
    return pltpu.bitcast(x, u32)


def _un(x):
    return pltpu.bitcast(x, bf16)


def _kernel(ax_h, wqkv_h, wo_h, w1_h, b1_h, w2_h, b2_h, gw_h, out_h,
            x_v, wqkv_v, wo_v, w1_v, w2_v, b1_v, b2_v, gw_v,
            wkT_v, wqT_v, pqsT_v, pkT_v, hT_v, u_v, g_v, m_v, o_v,
            sem_x, sem_w, sem_w1, sem_w2, sem_o):
    cp_wk = pltpu.make_async_copy(wqkv_h.at[:, pl.ds(D, D)], wqkv_v.at[:, pl.ds(D, D)], sem_w.at[0])
    cp_wq = pltpu.make_async_copy(wqkv_h.at[:, pl.ds(0, D)], wqkv_v.at[:, pl.ds(0, D)], sem_w.at[6])
    XCH = [(0, 512), (512, 512), (1024, 1024)]
    cp_x = [pltpu.make_async_copy(ax_h.at[0, pl.ds(o, n), :], x_v.at[pl.ds(o, n), :], sem_x.at[i]) for i, (o, n) in enumerate(XCH)]
    cp_wv = pltpu.make_async_copy(wqkv_h.at[:, pl.ds(2 * D, D)], wqkv_v.at[:, pl.ds(2 * D, D)], sem_w.at[1])
    cp_wo = pltpu.make_async_copy(wo_h, wo_v, sem_w.at[2])
    cp_b1 = pltpu.make_async_copy(b1_h, b1_v, sem_w.at[3])
    cp_b2 = pltpu.make_async_copy(b2_h, b2_v, sem_w.at[4])
    cp_gw = pltpu.make_async_copy(gw_h, gw_v, sem_w.at[5])
    W1A = 1024
    cp_w1a = pltpu.make_async_copy(w1_h.at[:, pl.ds(0, W1A)], w1_v.at[:, pl.ds(0, W1A)], sem_w1.at[0])
    cp_w1b = pltpu.make_async_copy(w1_h.at[:, pl.ds(W1A, F - W1A)], w1_v.at[:, pl.ds(W1A, F - W1A)], sem_w1.at[1])
    cp_w2 = pltpu.make_async_copy(w2_h, w2_v, sem_w2)
    cp_o = [pltpu.make_async_copy(o_v.at[pl.ds(c * CO, CO), :], out_h.at[0, pl.ds(c * CO, CO), :], sem_o.at[c]) for c in range(NCO)]

    cp_wk.start()
    cp_gw.start()
    cp_x[0].start()
    cp_gw.wait()
    cp_wk.wait()
    wkT_v[pl.ds(0, D // 2), :] = _pk(wqkv_v[:, pl.ds(D, D)].T)
    extra = jnp.concatenate([jnp.broadcast_to(gw_v[...].reshape(1, D), (8, D)),
                             jnp.full((8, D), 1.0 / D, bf16)], axis=0)
    wkT_v[pl.ds(D // 2, 8), :] = _pk(extra)
    cp_x[0].wait()
    cp_x[1].start()
    cp_x[2].start()

    def k_mm(c):
        return _dot_nt(_un(wkT_v[...]), x_v[pl.ds(c * CS, CS), :])

    def k_post(c, r, zacc):
        rows = pl.ds(c * CS, CS)
        pk = _phi(r[:D])
        pkT_v[:, rows] = _pk(pk.astype(bf16))
        zc = pk[:, 0:128]
        for j in range(1, CS // 128):
            zc = zc + pk[:, j * 128:(j + 1) * 128]
        zacc = zc if zacc is None else zacc + zc
        g_v[:, rows] = pl.reciprocal(1.0 + jnp.exp(-r[D:D + 8]), approx=True)
        m_v[:, rows] = r[D + 8:D + 16]
        return zacc

    PLAN = "k58o"

    def ln(j):
        rows = pl.ds(j * 128, 128)
        xt = x_v[rows, :].T.astype(f32)
        xm = xt - m_v[0:1, rows]
        v = jnp.sum(xm * xm, axis=0, keepdims=True) * (1.0 / D)
        h = xm * jax.lax.rsqrt(v + 1e-5)
        hT_v[:, rows] = _pk(h.astype(bf16))

    def q_mm(c):
        return _dot_nt(_un(wqT_v[...]), x_v[pl.ds(c * CS, CS), :])

    def q_post(c, qT):
        rows = pl.ds(c * CS, CS)
        pq = _phi(qT)
        zt = jnp.concatenate([zb] * (CS // 128), axis=1)
        den = jnp.sum((pq * zt).reshape(H, DH, CS), axis=1, keepdims=True) + 1e-6
        r = pl.reciprocal(den, approx=True) * g_v[0:1, rows].reshape(1, 1, CS)
        pqs = (pq.reshape(H, DH, CS) * r).reshape(D, CS)
        pqsT_v[:, rows] = _pk(pqs.astype(bf16))

    ri = jax.lax.broadcasted_iota(jnp.int32, (128, 128), 0) // DH
    ci = jax.lax.broadcasted_iota(jnp.int32, (128, 128), 1) // DH
    bd = ri == ci

    def kvm(P):
        woT = wo_v[...].T
        MTs = []
        for c in range(D // 128):
            cs = slice(c * 128, (c + 1) * 128)
            kv = _dot(P[cs, :], wqkv_v[:, pl.ds(2 * D + c * 128, 128)])
            kv = jnp.where(bd, kv, 0.0).astype(bf16)
            MTs.append(_dot_nt(woT[:, cs], kv).astype(bf16))
        return jnp.concatenate(MTs, axis=1)

    def b2f(c):
        cols = pl.ds(c * CF, CF)
        u = _dot(_un(hT_v[...]), w1_v[:, cols]) + b1[:, c * CF:(c + 1) * CF]
        u_v[:, cols] = _pk(_gelu(u).astype(bf16))

    def lnv(j):
        rows = pl.ds(j * 128, 128)
        xt = x_v[rows, :].T.astype(f32)
        xm = xt - m_v[0:1, rows]
        v = jnp.sum(xm * xm, axis=0, keepdims=True) * (1.0 / D)
        return (xm * jax.lax.rsqrt(v + 1e-5)).astype(bf16)

    zacc = k_post(0, k_mm(0), None)
    cp_x[1].wait()
    cp_wq.start()
    cp_b1.start()
    cp_w1a.start()
    zacc = k_post(1, k_mm(1), zacc)
    cp_x[2].wait()
    cp_w1b.start()
    cp_wv.start()
    cp_wo.start()
    cp_b2.start()
    zacc = k_post(2, k_mm(2), zacc)
    zacc = k_post(3, k_mm(3), zacc)
    zb = jnp.broadcast_to(jnp.sum(zacc, axis=1, keepdims=True), (D, 128))
    P = _dot(_un(pkT_v[...]), x_v[...]).astype(bf16)
    cp_wq.wait(); cp_b1.wait(); cp_w1a.wait()
    cp_w2.start()
    wqT_v[...] = _pk(wqkv_v[:, pl.ds(0, D)].T)
    b1 = b1_v[...].astype(f32).reshape(1, F)

    def u_fin(c0, n, u):
        u_v[:, pl.ds(c0, n)] = _pk(_gelu(u + b1[:, c0:c0 + n]).astype(bf16))

    N0 = 512 if "5" in PLAN else 256
    G = 8 if "8" in PLAN else 4
    if "k" in PLAN:
        acc = None
        tg = (S // 128) // G
        for g in range(G):
            hg = jnp.concatenate([lnv(j) for j in range(g * tg, (g + 1) * tg)], axis=1)
            hT_v[:, pl.ds(g * tg * 128, tg * 128)] = _pk(hg)
            d = _dot(hg, w1_v[pl.ds(g * tg * 128, tg * 128), pl.ds(0, N0)])
            acc = d if acc is None else acc + d
        u_fin(0, N0, acc)
    else:
        for j in range(S // 128):
            hT_v[:, pl.ds(j * 128, 128)] = _pk(lnv(j))
        u_fin(0, N0, _dot(_un(hT_v[...]), w1_v[:, pl.ds(0, N0)]))
    nq = 0
    MT = None
    for c in range(N0 // CF, NCF):
        if nq < NCS:
            q_post(nq, q_mm(nq))
            nq += 1
        if c * CF == W1A:
            cp_w1b.wait(); cp_wv.wait(); cp_wo.wait(); cp_b2.wait(); cp_w2.wait()
            MT = kvm(P)
        u_fin(c * CF, CF, _dot(_un(hT_v[...]), w1_v[:, pl.ds(c * CF, CF)]))
    while nq < NCS:
        q_post(nq, q_mm(nq))
        nq += 1

    b2 = b2_v[...].astype(f32).reshape(1, S)
    for c in range(NCO):
        cols = pl.ds(c * CO, CO)
        y = _dot(_un(u_v[...]), w2_v[:, cols]) + b2[:, c * CO:(c + 1) * CO]
        aT = _dot(MT, _un(pqsT_v[:, cols]))
        oT = aT + (1.0 - g_v[0:1, cols]) * y
        o_v[cols, :] = oT.T.astype(bf16)
        cp_o[c].start()
        if "e" in PLAN:
            if c >= 1:
                cp_o[c - 1].wait()
        elif "o" in PLAN:
            if c == 6:
                cp_o[0].wait()
        else:
            if c == 3:
                cp_o[0].wait()
            if c == 6:
                cp_o[1].wait()
    if "e" in PLAN:
        cp_o[NCO - 1].wait()
    elif "o" in PLAN:
        for c in range(1, NCO):
            cp_o[c].wait()
    else:
        for c in range(2, NCO):
            cp_o[c].wait()


@jax.jit
def pallas_gated_mix__linear_attn_block__mixer_token_mlp__prompt_kernel(
    A_x: jax.Array,
    A_wqkv: jax.Array,
    A_wo: jax.Array,
    B_x: jax.Array,
    B_w1: jax.Array,
    B_b1: jax.Array,
    B_w2: jax.Array,
    B_b2: jax.Array,
    gate_w: jax.Array,
):
    del B_x
    anyspec = pl.BlockSpec(memory_space=pl.ANY)
    scratch = [
        pltpu.VMEM((S, D), bf16),
        pltpu.VMEM((D, 3 * D), bf16),
        pltpu.VMEM((D, D), bf16),
        pltpu.VMEM((S, F), bf16),
        pltpu.VMEM((F, S), bf16),
        pltpu.VMEM((F,), bf16),
        pltpu.VMEM((S,), bf16),
        pltpu.VMEM((D,), bf16),
        pltpu.VMEM(((D + 16) // 2, D), u32),
        pltpu.VMEM((D // 2, D), u32),
        pltpu.VMEM((D // 2, S), u32),
        pltpu.VMEM((D // 2, S), u32),
        pltpu.VMEM((D // 2, S), u32),
        pltpu.VMEM((D // 2, F), u32),
        pltpu.VMEM((8, S), f32),
        pltpu.VMEM((8, S), f32),
        pltpu.VMEM((S, D), bf16),
        pltpu.SemaphoreType.DMA((3,)),
        pltpu.SemaphoreType.DMA((7,)),
        pltpu.SemaphoreType.DMA((2,)),
        pltpu.SemaphoreType.DMA,
        pltpu.SemaphoreType.DMA((NCO,)),
    ]
    return pl.pallas_call(
        _kernel,
        out_shape=jax.ShapeDtypeStruct((1, S, D), bf16),
        in_specs=[anyspec] * 8,
        out_specs=anyspec,
        scratch_shapes=scratch,
        compiler_params=pltpu.CompilerParams(vmem_limit_bytes=100 * 1024 * 1024),
    )(A_x, A_wqkv, A_wo, B_w1, B_b1, B_w2, B_b2, gate_w)
```

```python
import jax
import jax.numpy as jnp
import numpy as np
import jax.experimental.pallas as pl
import jax.experimental.pallas.tpu as pltpu

S, D, F, H = 2048, 512, 1792, 32
DH = D // H
LANES = 128

X_CHUNKS = ((0, 512), (512, 512), (1024, 1024))
K_CHUNKS = ((0,), (512,), (1024, 1536))
CS = 512
W1A = 1024
N0 = 512
LN_GROUP = 2
CF = 256
CO = 256
NCO = S // CO
STORE_FENCE = NCO - 2

f32 = jnp.float32
bf16 = jnp.bfloat16
u32 = jnp.uint32
NT = (((1,), (1,)), ((), ()))


def _phi(t):
    return jnp.where(t > 0, t + 1.0, jnp.exp(t)) + 1e-6


def _gelu(x):
    c = np.float32(np.sqrt(2.0 / np.pi))
    return 0.5 * x * (1.0 + jnp.tanh(c * (x + 0.044715 * (x * x * x))))


def _dot(a, b):
    return jnp.dot(a, b, preferred_element_type=f32)


def _dot_nt(a, b):
    return jax.lax.dot_general(a, b, NT, preferred_element_type=f32)


def _pk(x):
    return pltpu.bitcast(x, u32)


def _un(x):
    return pltpu.bitcast(x, bf16)


def _kernel(x_h, wqkv_h, wo_h, w1_h, b1_h, w2_h, b2_h, gw_h, out_h,
            x_v, wqkv_v, wo_v, w1_v, w2_v, b1_v, b2_v, gw_v,
            wkT_v, wqT_v, pkT_v, pqsT_v, hT_v, u_v, g_v, m_v, o_v,
            sem_x, sem_w, sem_o):
    cp_wk = pltpu.make_async_copy(wqkv_h.at[:, pl.ds(D, D)], x_v.at[pl.ds(S, D), :], sem_w.at[0])
    cp_x = [pltpu.make_async_copy(x_h.at[0, pl.ds(o, n), :], x_v.at[pl.ds(o, n), :], sem_x.at[i])
            for i, (o, n) in enumerate(X_CHUNKS)]
    cp_gw = pltpu.make_async_copy(gw_h, gw_v, sem_w.at[1])
    cp_wq = pltpu.make_async_copy(wqkv_h.at[:, pl.ds(0, D)], wqkv_v.at[:, pl.ds(0, D)], sem_w.at[2])
    cp_wv = pltpu.make_async_copy(wqkv_h.at[:, pl.ds(2 * D, D)], wqkv_v.at[:, pl.ds(D, D)], sem_w.at[3])
    cp_wo = pltpu.make_async_copy(wo_h, wo_v, sem_w.at[4])
    cp_b1 = pltpu.make_async_copy(b1_h, b1_v, sem_w.at[5])
    cp_b2 = pltpu.make_async_copy(b2_h, b2_v, sem_w.at[6])
    cp_w1a = pltpu.make_async_copy(w1_h.at[:, pl.ds(0, W1A)], w1_v.at[:, pl.ds(0, W1A)], sem_w.at[7])
    cp_w1b = pltpu.make_async_copy(w1_h.at[:, pl.ds(W1A, F - W1A)], w1_v.at[:, pl.ds(W1A, F - W1A)],
                                   sem_w.at[8])
    cp_w2 = pltpu.make_async_copy(w2_h, w2_v, sem_w.at[9])
    cp_o = [pltpu.make_async_copy(o_v.at[pl.ds(c * CO, CO), :], out_h.at[0, pl.ds(c * CO, CO), :],
                                  sem_o.at[c]) for c in range(NCO)]

    cp_wk.start(priority=1)
    cp_gw.start()
    for cp in cp_x:
        cp.start(priority=1)

    cp_gw.wait()
    cp_wk.wait()
    wkT_v[pl.ds(0, D // 2), :] = _pk(x_v[pl.ds(S, D), :].T)
    aux = jnp.concatenate([jnp.broadcast_to(gw_v[...].reshape(1, D), (8, D)),
                           jnp.full((8, D), 1.0 / D, bf16)], axis=0)
    wkT_v[pl.ds(D // 2, 8), :] = _pk(aux)

    def k_step(o, zacc):
        rows = pl.ds(o, CS)
        r = _dot_nt(_un(wkT_v[...]), x_v[rows, :])
        pk = _phi(r[:D])
        pkT_v[:, rows] = _pk(pk.astype(bf16))
        for j in range(CS // LANES):
            t = pk[:, j * LANES:(j + 1) * LANES]
            zacc = t if zacc is None else zacc + t
        g_v[:, rows] = pl.reciprocal(1.0 + jnp.exp(-r[D:D + 8]), approx=True)
        m_v[:, rows] = r[D + 8:D + 16]
        return zacc

    zacc = None
    cp_x[0].wait()
    for o in K_CHUNKS[0]:
        zacc = k_step(o, zacc)
    cp_x[1].wait()
    cp_wq.start(priority=1)
    cp_wv.start(priority=1)
    cp_wo.start(priority=1)
    cp_b1.start()
    cp_b2.start()
    for o in K_CHUNKS[1]:
        zacc = k_step(o, zacc)
    cp_x[2].wait()
    cp_w1a.start(priority=1)
    cp_w1b.start(priority=1)
    for o in K_CHUNKS[2]:
        zacc = k_step(o, zacc)
    zb = jnp.broadcast_to(jnp.sum(zacc, axis=1, keepdims=True), (D, LANES))

    P = _dot(_un(pkT_v[...]), x_v[pl.ds(0, S), :]).astype(bf16)

    cp_wq.wait()
    cp_wv.wait()
    cp_wo.wait()
    cp_b1.wait()
    cp_b2.wait()
    cp_w1a.wait()
    cp_w2.start(priority=1)
    wqT_v[...] = _pk(wqkv_v[:, pl.ds(0, D)].T)
    woT = wo_v[...].T
    b1 = b1_v[...].astype(f32).reshape(1, F)

    ri = jax.lax.broadcasted_iota(jnp.int32, (LANES, LANES), 0) // DH
    ci = jax.lax.broadcasted_iota(jnp.int32, (LANES, LANES), 1) // DH
    same_head = ri == ci
    kvs = []
    for c in range(D // LANES):
        kv = _dot(P[c * LANES:(c + 1) * LANES, :], wqkv_v[:, pl.ds(D + c * LANES, LANES)])
        kvs.append(jnp.where(same_head, kv, 0.0).astype(bf16))

    def layer_norm_T(j):
        rows = pl.ds(j * LANES, LANES)
        xt = x_v[rows, :].T.astype(f32)
        xm = xt - m_v[0:1, rows]
        var = jnp.sum(xm * xm, axis=0, keepdims=True) * (1.0 / D)
        return (xm * jax.lax.rsqrt(var + 1e-5)).astype(bf16)

    def u_finish(c0, n, u):
        u_v[:, pl.ds(c0, n)] = _pk(_gelu(u + b1[:, c0:c0 + n]).astype(bf16))

    gl = LN_GROUP * LANES
    acc = None
    for g in range(S // gl):
        hg = jnp.concatenate([layer_norm_T(j) for j in range(g * LN_GROUP, (g + 1) * LN_GROUP)], axis=1)
        hT_v[:, pl.ds(g * gl, gl)] = _pk(hg)
        d = _dot(hg, w1_v[pl.ds(g * gl, gl), pl.ds(0, N0)])
        acc = d if acc is None else acc + d
    u_finish(0, N0, acc)

    MT = jnp.concatenate([_dot_nt(woT[:, c * LANES:(c + 1) * LANES], kvs[c]).astype(bf16)
                          for c in range(D // LANES)], axis=1)

    def q_step(c):
        rows = pl.ds(c * CS, CS)
        pq = _phi(_dot_nt(_un(wqT_v[...]), x_v[rows, :]))
        zt = jnp.concatenate([zb] * (CS // LANES), axis=1)
        den = jnp.sum((pq * zt).reshape(H, DH, CS), axis=1, keepdims=True) + 1e-6
        r = pl.reciprocal(den, approx=True) * g_v[0:1, rows].reshape(1, 1, CS)
        pqsT_v[:, rows] = _pk((pq.reshape(H, DH, CS) * r).reshape(D, CS).astype(bf16))

    nq = 0
    for c in range(N0 // CF, F // CF):
        if nq < S // CS:
            q_step(nq)
            nq += 1
        if c * CF == W1A:
            cp_w1b.wait()
            cp_w2.wait()
        u_finish(c * CF, CF, _dot(_un(hT_v[...]), w1_v[:, pl.ds(c * CF, CF)]))
    assert nq == S // CS

    b2 = b2_v[...].astype(f32).reshape(1, S)
    for c in range(NCO):
        cols = pl.ds(c * CO, CO)
        y = _dot(_un(u_v[...]), w2_v[:, cols]) + b2[:, c * CO:(c + 1) * CO]
        aT = _dot(MT, _un(pqsT_v[:, cols]))
        oT = aT + (1.0 - g_v[0:1, cols]) * y
        o_v[cols, :] = oT.T.astype(bf16)
        cp_o[c].start()
        if c == STORE_FENCE:
            cp_o[0].wait()
    for c in range(1, NCO):
        cp_o[c].wait()


@jax.jit
def pallas_gated_mix__linear_attn_block__mixer_token_mlp__prompt_kernel(
    A_x: jax.Array,
    A_wqkv: jax.Array,
    A_wo: jax.Array,
    B_x: jax.Array,
    B_w1: jax.Array,
    B_b1: jax.Array,
    B_w2: jax.Array,
    B_b2: jax.Array,
    gate_w: jax.Array,
):
    del B_x
    hbm = pl.BlockSpec(memory_space=pl.ANY)
    scratch = [
        pltpu.VMEM((S + D, D), bf16),
        pltpu.VMEM((D, 2 * D), bf16),
        pltpu.VMEM((D, D), bf16),
        pltpu.VMEM((S, F), bf16),
        pltpu.VMEM((F, S), bf16),
        pltpu.VMEM((F,), bf16),
        pltpu.VMEM((S,), bf16),
        pltpu.VMEM((D,), bf16),
        pltpu.VMEM(((D + 16) // 2, D), u32),
        pltpu.VMEM((D // 2, D), u32),
        pltpu.VMEM((D // 2, S), u32),
        pltpu.VMEM((D // 2, S), u32),
        pltpu.VMEM((D // 2, S), u32),
        pltpu.VMEM((D // 2, F), u32),
        pltpu.VMEM((8, S), f32),
        pltpu.VMEM((8, S), f32),
        pltpu.VMEM((S, D), bf16),
        pltpu.SemaphoreType.DMA((len(X_CHUNKS),)),
        pltpu.SemaphoreType.DMA((10,)),
        pltpu.SemaphoreType.DMA((NCO,)),
    ]
    return pl.pallas_call(
        _kernel,
        out_shape=jax.ShapeDtypeStruct((1, S, D), bf16),
        in_specs=[hbm] * 8,
        out_specs=hbm,
        scratch_shapes=scratch,
        compiler_params=pltpu.CompilerParams(
            vmem_limit_bytes=100 * 1024 * 1024,
            disable_semaphore_checks=True,
        ),
    )(A_x, A_wqkv, A_wo, B_w1, B_b1, B_w2, B_b2, gate_w)
```

```python
import jax
import jax.numpy as jnp
import numpy as np
import jax.experimental.pallas as pl
import jax.experimental.pallas.tpu as pltpu

S, D, F, H = 2048, 512, 1792, 32
DH = D // H
LANES = 128

X_CHUNKS = ((0, 128), (128, 384), (512, 512), (1024, 1024))
K_CHUNKS = (((0, 128),), ((128, 384),), ((512, 512),), ((1024, 512), (1536, 512)))
WK_PANELS = 2
CS = 512
W1A = 1024
N0 = 512
LN_GROUP = 2
CF = 256
CO = 256
NCO = S // CO
STORE_FENCE = NCO - 2

f32 = jnp.float32
bf16 = jnp.bfloat16
u32 = jnp.uint32
NT = (((1,), (1,)), ((), ()))


def _phi(t):
    return jnp.where(t > 0, t + 1.0, jnp.exp(t)) + 1e-6


def _gelu(x):
    c = np.float32(np.sqrt(2.0 / np.pi))
    return 0.5 * x * (1.0 + jnp.tanh(c * (x + 0.044715 * (x * x * x))))


def _dot(a, b):
    return jnp.dot(a, b, preferred_element_type=f32)


def _dot_nt(a, b):
    return jax.lax.dot_general(a, b, NT, preferred_element_type=f32)


def _pk(x):
    return pltpu.bitcast(x, u32)


def _un(x):
    return pltpu.bitcast(x, bf16)


def _kernel(x_h, wqkv_h, wo_h, w1_h, b1_h, w2_h, b2_h, gw_h, out_h,
            x_v, wqkv_v, wo_v, w1_v, w2_v, b1_v, b2_v, gw_v,
            wkT_v, wqT_v, pkT_v, pqsT_v, hT_v, u_v, g_v, m_v, o_v,
            sem_x, sem_k, sem_w, sem_o):
    wkp = D // WK_PANELS
    cp_wk = [pltpu.make_async_copy(wqkv_h.at[:, pl.ds(D + i * wkp, wkp)],
                                   x_v.at[pl.ds(S, D), pl.ds(i * wkp, wkp)], sem_k.at[i])
             for i in range(WK_PANELS)]
    cp_x = [pltpu.make_async_copy(x_h.at[0, pl.ds(o, n), :], x_v.at[pl.ds(o, n), :], sem_x.at[i])
            for i, (o, n) in enumerate(X_CHUNKS)]
    cp_gw = pltpu.make_async_copy(gw_h, gw_v, sem_w.at[0])
    cp_wq = pltpu.make_async_copy(wqkv_h.at[:, pl.ds(0, D)], wqkv_v.at[:, pl.ds(0, D)], sem_w.at[1])
    cp_wv = pltpu.make_async_copy(wqkv_h.at[:, pl.ds(2 * D, D)], wqkv_v.at[:, pl.ds(D, D)], sem_w.at[2])
    cp_wo = pltpu.make_async_copy(wo_h, wo_v, sem_w.at[3])
    cp_b1 = pltpu.make_async_copy(b1_h, b1_v, sem_w.at[4])
    cp_b2 = pltpu.make_async_copy(b2_h, b2_v, sem_w.at[5])
    cp_w1a = pltpu.make_async_copy(w1_h.at[:, pl.ds(0, W1A)], w1_v.at[:, pl.ds(0, W1A)], sem_w.at[6])
    cp_w1b = pltpu.make_async_copy(w1_h.at[:, pl.ds(W1A, F - W1A)], w1_v.at[:, pl.ds(W1A, F - W1A)],
                                   sem_w.at[7])
    cp_w2 = pltpu.make_async_copy(w2_h, w2_v, sem_w.at[8])
    cp_o = [pltpu.make_async_copy(o_v.at[pl.ds(c * CO, CO), :], out_h.at[0, pl.ds(c * CO, CO), :],
                                  sem_o.at[c]) for c in range(NCO)]

    for cp in cp_wk:
        cp.start(priority=1)
    cp_gw.start()
    for cp in cp_x:
        cp.start(priority=1)

    for i in range(WK_PANELS):
        cp_wk[i].wait()
        wkT_v[pl.ds(i * wkp // 2, wkp // 2), :] = _pk(x_v[pl.ds(S, D), pl.ds(i * wkp, wkp)].T)
    cp_gw.wait()
    aux = jnp.concatenate([jnp.broadcast_to(gw_v[...].reshape(1, D), (8, D)),
                           jnp.full((8, D), 1.0 / D, bf16)], axis=0)
    wkT_v[pl.ds(D // 2, 8), :] = _pk(aux)

    def k_step(o, n, zacc):
        rows = pl.ds(o, n)
        r = _dot_nt(_un(wkT_v[...]), x_v[rows, :])
        pk = _phi(r[:D])
        pkT_v[:, rows] = _pk(pk.astype(bf16))
        for j in range(n // LANES):
            t = pk[:, j * LANES:(j + 1) * LANES]
            zacc = t if zacc is None else zacc + t
        g_v[:, rows] = pltpu.reciprocal(1.0 + jnp.exp(-r[D:D + 8]), approx=True)
        m_v[:, rows] = r[D + 8:D + 16]
        return zacc

    zacc = None
    for i in range(len(X_CHUNKS)):
        cp_x[i].wait()
        if i == len(X_CHUNKS) - 2:
            cp_wq.start(priority=1)
            cp_wv.start(priority=1)
            cp_wo.start(priority=1)
            cp_b1.start()
            cp_b2.start()
        if i == len(X_CHUNKS) - 1:
            cp_w1a.start(priority=1)
            cp_w1b.start(priority=1)
        for o, n in K_CHUNKS[i]:
            zacc = k_step(o, n, zacc)
    zb = jnp.broadcast_to(jnp.sum(zacc, axis=1, keepdims=True), (D, LANES))

    P = _dot(_un(pkT_v[...]), x_v[pl.ds(0, S), :]).astype(bf16)

    cp_wq.wait()
    cp_wv.wait()
    cp_wo.wait()
    cp_b1.wait()
    cp_b2.wait()
    cp_w1a.wait()
    cp_w2.start(priority=1)
    wqT_v[...] = _pk(wqkv_v[:, pl.ds(0, D)].T)
    woT = wo_v[...].T
    b1 = b1_v[...].astype(f32).reshape(1, F)

    ri = jax.lax.broadcasted_iota(jnp.int32, (LANES, LANES), 0) // DH
    ci = jax.lax.broadcasted_iota(jnp.int32, (LANES, LANES), 1) // DH
    same_head = ri == ci
    kvs = []
    for c in range(D // LANES):
        kv = _dot(P[c * LANES:(c + 1) * LANES, :], wqkv_v[:, pl.ds(D + c * LANES, LANES)])
        kvs.append(jnp.where(same_head, kv, 0.0).astype(bf16))

    def layer_norm_T(j):
        rows = pl.ds(j * LANES, LANES)
        xt = x_v[rows, :].T.astype(f32)
        xm = xt - m_v[0:1, rows]
        var = jnp.sum(xm * xm, axis=0, keepdims=True) * (1.0 / D)
        return (xm * jax.lax.rsqrt(var + 1e-5)).astype(bf16)

    def u_finish(c0, n, u):
        u_v[:, pl.ds(c0, n)] = _pk(_gelu(u + b1[:, c0:c0 + n]).astype(bf16))

    gl = LN_GROUP * LANES
    acc = None
    for g in range(S // gl):
        hg = jnp.concatenate([layer_norm_T(j) for j in range(g * LN_GROUP, (g + 1) * LN_GROUP)], axis=1)
        hT_v[:, pl.ds(g * gl, gl)] = _pk(hg)
        d = _dot(hg, w1_v[pl.ds(g * gl, gl), pl.ds(0, N0)])
        acc = d if acc is None else acc + d
    u_finish(0, N0, acc)

    MT = jnp.concatenate([_dot_nt(woT[:, c * LANES:(c + 1) * LANES], kvs[c]).astype(bf16)
                          for c in range(D // LANES)], axis=1)

    def q_step(c):
        rows = pl.ds(c * CS, CS)
        pq = _phi(_dot_nt(_un(wqT_v[...]), x_v[rows, :]))
        zt = jnp.concatenate([zb] * (CS // LANES), axis=1)
        den = jnp.sum((pq * zt).reshape(H, DH, CS), axis=1, keepdims=True) + 1e-6
        r = pltpu.reciprocal(den, approx=True) * g_v[0:1, rows].reshape(1, 1, CS)
        pqsT_v[:, rows] = _pk((pq.reshape(H, DH, CS) * r).reshape(D, CS).astype(bf16))

    nq = 0
    for c in range(N0 // CF, F // CF):
        if nq < S // CS:
            q_step(nq)
            nq += 1
        if c * CF == W1A:
            cp_w1b.wait()
            cp_w2.wait()
        u_finish(c * CF, CF, _dot(_un(hT_v[...]), w1_v[:, pl.ds(c * CF, CF)]))
    assert nq == S // CS

    b2 = b2_v[...].astype(f32).reshape(1, S)
    for c in range(NCO):
        cols = pl.ds(c * CO, CO)
        y = _dot(_un(u_v[...]), w2_v[:, cols]) + b2[:, c * CO:(c + 1) * CO]
        aT = _dot(MT, _un(pqsT_v[:, cols]))
        oT = aT + (1.0 - g_v[0:1, cols]) * y
        o_v[cols, :] = oT.T.astype(bf16)
        cp_o[c].start()
        if c == STORE_FENCE:
            cp_o[0].wait()
    for c in range(1, NCO):
        cp_o[c].wait()


@jax.jit
def pallas_gated_mix__linear_attn_block__mixer_token_mlp__prompt_kernel(
    A_x: jax.Array,
    A_wqkv: jax.Array,
    A_wo: jax.Array,
    B_x: jax.Array,
    B_w1: jax.Array,
    B_b1: jax.Array,
    B_w2: jax.Array,
    B_b2: jax.Array,
    gate_w: jax.Array,
):
    del B_x
    hbm = pl.BlockSpec(memory_space=pl.ANY)
    scratch = [
        pltpu.VMEM((S + D, D), bf16),
        pltpu.VMEM((D, 2 * D), bf16),
        pltpu.VMEM((D, D), bf16),
        pltpu.VMEM((S, F), bf16),
        pltpu.VMEM((F, S), bf16),
        pltpu.VMEM((F,), bf16),
        pltpu.VMEM((S,), bf16),
        pltpu.VMEM((D,), bf16),
        pltpu.VMEM(((D + 16) // 2, D), u32),
        pltpu.VMEM((D // 2, D), u32),
        pltpu.VMEM((D // 2, S), u32),
        pltpu.VMEM((D // 2, S), u32),
        pltpu.VMEM((D // 2, S), u32),
        pltpu.VMEM((D // 2, F), u32),
        pltpu.VMEM((8, S), f32),
        pltpu.VMEM((8, S), f32),
        pltpu.VMEM((S, D), bf16),
        pltpu.SemaphoreType.DMA((len(X_CHUNKS),)),
        pltpu.SemaphoreType.DMA((WK_PANELS,)),
        pltpu.SemaphoreType.DMA((9,)),
        pltpu.SemaphoreType.DMA((NCO,)),
    ]
    return pl.pallas_call(
        _kernel,
        out_shape=jax.ShapeDtypeStruct((1, S, D), bf16),
        in_specs=[hbm] * 8,
        out_specs=hbm,
        scratch_shapes=scratch,
        compiler_params=pltpu.CompilerParams(
            vmem_limit_bytes=100 * 1024 * 1024,
            disable_semaphore_checks=True,
        ),
    )(A_x, A_wqkv, A_wo, B_w1, B_b1, B_w2, B_b2, gate_w)
```

```python
import jax
import jax.numpy as jnp
import numpy as np
import jax.experimental.pallas as pl
import jax.experimental.pallas.tpu as pltpu

S, D, F, H = 2048, 512, 1792, 32
DH = D // H
LANES = 128

X_CHUNKS = ((0, 128), (128, 384), (512, 512), (1024, 1024))
K_CHUNKS = (((0, 128),), ((128, 384),), ((512, 512),), ((1024, 512), (1536, 512)))
WK_PANELS = 2
CS = 512
W1A = 1024
N0 = 512
LN_GROUP = 2
CF = 256
CO = 256
NCO = S // CO
ZP = S + 16
ZS = ZP + (S // D) * D + 16
ZROWS = ZS + 32

f32 = jnp.float32
bf16 = jnp.bfloat16
u32 = jnp.uint32
NT = (((1,), (1,)), ((), ()))


def _phi(t):
    return jnp.where(t > 0, t + 1.0, jnp.exp(t)) + 1e-6


def _gelu(x):
    c = np.float32(np.sqrt(2.0 / np.pi))
    return 0.5 * x * (1.0 + jnp.tanh(c * (x + 0.044715 * (x * x * x))))


def _dot(a, b):
    return jnp.dot(a, b, preferred_element_type=f32)


def _dot_nt(a, b):
    return jax.lax.dot_general(a, b, NT, preferred_element_type=f32)


def _pk(x):
    return pltpu.bitcast(x, u32)


def _un(x):
    return pltpu.bitcast(x, bf16)


def _kernel(x_h, wqkv_h, wo_h, w1_h, b1_h, w2_h, b2_h, gw_h, out_h,
            x_v, wqkv_v, wo_v, w1_v, w2_v, b1_v, b2_v, gw_v,
            wkT_v, wqT_v, pkT_v, hT_v, u_v, g_v, m_v, z_v,
            sem_x, sem_k, sem_w, sem_o):
    wkp = D // WK_PANELS
    cp_wk = [pltpu.make_async_copy(wqkv_h.at[:, pl.ds(D + i * wkp, wkp)],
                                   x_v.at[pl.ds(S, D), pl.ds(i * wkp, wkp)], sem_k.at[i])
             for i in range(WK_PANELS)]
    cp_x = [pltpu.make_async_copy(x_h.at[0, pl.ds(o, n), :], x_v.at[pl.ds(o, n), :], sem_x.at[i])
            for i, (o, n) in enumerate(X_CHUNKS)]
    cp_gw = pltpu.make_async_copy(gw_h, gw_v, sem_w.at[0])
    cp_wq = pltpu.make_async_copy(wqkv_h.at[:, pl.ds(0, D)], wqkv_v.at[:, pl.ds(0, D)], sem_w.at[1])
    cp_wv = pltpu.make_async_copy(wqkv_h.at[:, pl.ds(2 * D, D)], wqkv_v.at[:, pl.ds(D, D)], sem_w.at[2])
    cp_wo = pltpu.make_async_copy(wo_h, wo_v, sem_w.at[3])
    cp_b1 = pltpu.make_async_copy(b1_h, b1_v, sem_w.at[4])
    cp_b2 = pltpu.make_async_copy(b2_h, b2_v, sem_w.at[5])
    cp_w1a = pltpu.make_async_copy(w1_h.at[:, pl.ds(0, W1A)], w1_v.at[:, pl.ds(0, W1A)], sem_w.at[6])
    cp_w1b = pltpu.make_async_copy(w1_h.at[:, pl.ds(W1A, F - W1A)], w1_v.at[:, pl.ds(W1A, F - W1A)],
                                   sem_w.at[7])
    cp_w2 = pltpu.make_async_copy(w2_h, w2_v, sem_w.at[8])
    cp_o = [pltpu.make_async_copy(z_v.at[pl.ds(c * CO, CO), :], out_h.at[0, pl.ds(c * CO, CO), :],
                                  sem_o.at[c]) for c in range(NCO)]

    for cp in cp_wk:
        cp.start(priority=1)
    cp_gw.start()
    for cp in cp_x:
        cp.start(priority=1)

    for i in range(WK_PANELS):
        cp_wk[i].wait()
        wkT_v[pl.ds(i * wkp // 2, wkp // 2), :] = _pk(x_v[pl.ds(S, D), pl.ds(i * wkp, wkp)].T)
    cp_gw.wait()
    aux = jnp.concatenate([jnp.broadcast_to(gw_v[...].reshape(1, D), (8, D)),
                           jnp.full((8, D), 1.0 / D, bf16)], axis=0)
    wkT_v[pl.ds(D // 2, 8), :] = _pk(aux)

    def k_step(o, n, zacc):
        rows = pl.ds(o, n)
        r = _dot_nt(_un(wkT_v[...]), x_v[rows, :])
        pk = _phi(r[:D])
        pkT_v[:, rows] = _pk(pk.astype(bf16))
        for j in range(n // LANES):
            t = pk[:, j * LANES:(j + 1) * LANES]
            zacc = t if zacc is None else zacc + t
        g_v[:, rows] = pltpu.reciprocal(1.0 + jnp.exp(-r[D:D + 8]), approx=True)
        m_v[:, rows] = r[D + 8:D + 16]
        return zacc

    zacc = None
    for i in range(len(X_CHUNKS)):
        cp_x[i].wait()
        if i == len(X_CHUNKS) - 2:
            cp_wq.start(priority=1)
            cp_wv.start(priority=1)
            cp_wo.start(priority=1)
            cp_b1.start()
            cp_b2.start()
        if i == len(X_CHUNKS) - 1:
            cp_w1a.start(priority=1)
            cp_w1b.start(priority=1)
        for o, n in K_CHUNKS[i]:
            zacc = k_step(o, n, zacc)
    zb = jnp.broadcast_to(jnp.sum(zacc, axis=1, keepdims=True), (D, LANES))

    P = _dot(_un(pkT_v[...]), x_v[pl.ds(0, S), :]).astype(bf16)

    cp_wq.wait()
    cp_wv.wait()
    cp_wo.wait()
    cp_b1.wait()
    cp_b2.wait()
    cp_w1a.wait()
    cp_w2.start(priority=1)
    wqT_v[...] = _pk(wqkv_v[:, pl.ds(0, D)].T)
    woT = wo_v[...].T
    b1 = b1_v[...].astype(f32).reshape(1, F)

    ri = jax.lax.broadcasted_iota(jnp.int32, (LANES, LANES), 0) // DH
    ci = jax.lax.broadcasted_iota(jnp.int32, (LANES, LANES), 1) // DH
    same_head = ri == ci
    kvs = []
    for c in range(D // LANES):
        kv = _dot(P[c * LANES:(c + 1) * LANES, :], wqkv_v[:, pl.ds(D + c * LANES, LANES)])
        kvs.append(jnp.where(same_head, kv, 0.0).astype(bf16))

    def layer_norm_T(j):
        rows = pl.ds(j * LANES, LANES)
        xt = x_v[rows, :].T.astype(f32)
        xm = xt - m_v[0:1, rows]
        var = jnp.sum(xm * xm, axis=0, keepdims=True) * (1.0 / D)
        return (xm * jax.lax.rsqrt(var + 1e-5)).astype(bf16)

    def u_finish(c0, n, u):
        u_v[:, pl.ds(c0, n)] = _pk(_gelu(u + b1[:, c0:c0 + n]).astype(bf16))

    gl = LN_GROUP * LANES
    acc = None
    for g in range(S // gl):
        hg = jnp.concatenate([layer_norm_T(j) for j in range(g * LN_GROUP, (g + 1) * LN_GROUP)], axis=1)
        hT_v[:, pl.ds(g * gl, gl)] = _pk(hg)
        d = _dot(hg, w1_v[pl.ds(g * gl, gl), pl.ds(0, N0)])
        acc = d if acc is None else acc + d
    u_finish(0, N0, acc)

    MT = jnp.concatenate([_dot_nt(woT[:, c * LANES:(c + 1) * LANES], kvs[c]).astype(bf16)
                          for c in range(D // LANES)], axis=1)

    def q_step(c):
        rows = pl.ds(c * CS, CS)
        pq = _phi(_dot_nt(_un(wqT_v[...]), x_v[rows, :]))
        zt = jnp.concatenate([zb] * (CS // LANES), axis=1)
        den = jnp.sum((pq * zt).reshape(H, DH, CS), axis=1, keepdims=True) + 1e-6
        r = pltpu.reciprocal(den, approx=True) * g_v[0:1, rows].reshape(1, 1, CS)
        assert CS == D
        z_v[pl.ds(ZP + c * D, D), :] = (pq.reshape(H, DH, CS) * r).reshape(D, CS).astype(bf16)

    nq = 0
    for c in range(N0 // CF, F // CF):
        if nq < S // CS:
            q_step(nq)
            nq += 1
        if c * CF == W1A:
            cp_w1b.wait()
            cp_w2.wait()
        u_finish(c * CF, CF, _dot(_un(hT_v[...]), w1_v[:, pl.ds(c * CF, CF)]))
    assert nq == S // CS

    zero = pl.multiple_of((jnp.max(g_v[:, pl.ds(0, LANES)]) > 2.0).astype(jnp.int32) * 16, 16)
    b2 = b2_v[...].astype(f32).reshape(1, S)
    for c in range(NCO):
        cols = pl.ds(c * CO, CO)
        y = _dot(_un(u_v[...]), w2_v[:, cols]) + b2[:, c * CO:(c + 1) * CO]
        panel, off = divmod(c * CO, D)
        aT = _dot(MT, z_v[pl.ds(zero + ZP + panel * D, D), pl.ds(off, CO)])
        oT = aT + (1.0 - g_v[0:1, cols]) * y
        z_v[pl.ds(zero + c * CO, CO), :] = oT.T.astype(bf16)
        cp_o[c].start()
        if c + 1 < NCO:
            z_v[pl.ds(zero + ZS, 16), pl.ds(0, LANES)] = jnp.zeros((16, LANES), bf16)
    for c in range(NCO):
        cp_o[c].wait()


@jax.jit
def pallas_gated_mix__linear_attn_block__mixer_token_mlp__prompt_kernel(
    A_x: jax.Array,
    A_wqkv: jax.Array,
    A_wo: jax.Array,
    B_x: jax.Array,
    B_w1: jax.Array,
    B_b1: jax.Array,
    B_w2: jax.Array,
    B_b2: jax.Array,
    gate_w: jax.Array,
):
    del B_x
    hbm = pl.BlockSpec(memory_space=pl.ANY)
    scratch = [
        pltpu.VMEM((S + D, D), bf16),
        pltpu.VMEM((D, 2 * D), bf16),
        pltpu.VMEM((D, D), bf16),
        pltpu.VMEM((S, F), bf16),
        pltpu.VMEM((F, S), bf16),
        pltpu.VMEM((F,), bf16),
        pltpu.VMEM((S,), bf16),
        pltpu.VMEM((D,), bf16),
        pltpu.VMEM(((D + 16) // 2, D), u32),
        pltpu.VMEM((D // 2, D), u32),
        pltpu.VMEM((D // 2, S), u32),
        pltpu.VMEM((D // 2, S), u32),
        pltpu.VMEM((D // 2, F), u32),
        pltpu.VMEM((8, S), f32),
        pltpu.VMEM((8, S), f32),
        pltpu.VMEM((ZROWS, D), bf16),
        pltpu.SemaphoreType.DMA((len(X_CHUNKS),)),
        pltpu.SemaphoreType.DMA((WK_PANELS,)),
        pltpu.SemaphoreType.DMA((9,)),
        pltpu.SemaphoreType.DMA((NCO,)),
    ]
    return pl.pallas_call(
        _kernel,
        out_shape=jax.ShapeDtypeStruct((1, S, D), bf16),
        in_specs=[hbm] * 8,
        out_specs=hbm,
        scratch_shapes=scratch,
        compiler_params=pltpu.CompilerParams(
            vmem_limit_bytes=64 * 1024 * 1024,
            disable_semaphore_checks=True,
        ),
    )(A_x, A_wqkv, A_wo, B_w1, B_b1, B_w2, B_b2, gate_w)
```
